```python
import os as _os
_os.environ.setdefault("JAX_PLATFORMS", "cpu")
import jax
import jax.numpy as jnp

def _softmax(x, axis=-1):
    return jax.nn.softmax(x, axis=axis)
def _gelu(x):
    return jax.nn.gelu(x, approximate=True)
def _silu(x):
    return jax.nn.silu(x)
def _sigmoid(x):
    return jax.nn.sigmoid(x)
def _layernorm(x, axis=-1, eps=1e-5):
    m = jnp.mean(x, axis=axis, keepdims=True)
    v = jnp.var(x, axis=axis, keepdims=True)
    return (x - m) / jnp.sqrt(v + eps)
def _scatter_add(tgt, idx, src, axis=0):
    return tgt.at[idx].add(src)
def _segment_sum(src, seg, n):
    return jax.ops.segment_sum(src, seg, n)
class _Rng:
    def __init__(self, key):
        self._k = key
    def _next(self):
        self._k, sub = jax.random.split(self._k)
        return sub
    def normal(self, shape):
        return jax.random.normal(self._next(), shape, dtype=jnp.bfloat16)
    def randint(self, lo, hi, shape):
        return jax.random.randint(self._next(), shape, lo, hi, dtype=jnp.int32)
    def uniform(self, shape, lo=0.0, hi=1.0):
        return jax.random.uniform(self._next(), shape, jnp.bfloat16, lo, hi)
    def permutation(self, n):
        return jax.random.permutation(self._next(), n)


kernel_name = 'parallel_sum__softmax_full_mha__swiglu_ffn__prompt'

def setup_inputs():
    _rng = _Rng(jax.random.key(int.from_bytes(__import__("os").urandom(4), "little")))
    _w = (lambda a: (lambda t: t.astype(jnp.bfloat16) if jnp.issubdtype(t.dtype, jnp.floating) else t)(jnp.asarray(a)))
    def _A_setup():
        B, S, D = 1, 2048, 640
        return {
            "x": _w((lambda *s: _rng.normal(s) * 0.05)(B, S, D)),
            "wqkv": _w((lambda *s: _rng.normal(s) * 0.1)(D, 3 * D)),
            "wo": _w((lambda *s: _rng.normal(s) * 0.05)(D, D)),
        }
    _A_in = _A_setup()

    def _B_setup():
        B, S, D, F = 1, 2048, 640, 1536
        return {
            "x": _w((lambda *s: _rng.normal(s) * 0.05)(B, S, D)),
            "w_gate": _w((lambda *s: _rng.normal(s) * 0.05)(D, F)),
            "w_up": _w((lambda *s: _rng.normal(s) * 0.05)(D, F)),
            "w_down": _w((lambda *s: _rng.normal(s) * 0.05)(F, D)),
        }
    _B_in = _B_setup()

    return {
        "A_x": _A_in["x"],
        "A_wqkv": _A_in["wqkv"],
        "A_wo": _A_in["wo"],
        "B_x": _B_in["x"],
        "B_w_gate": _B_in["w_gate"],
        "B_w_up": _B_in["w_up"],
        "B_w_down": _B_in["w_down"],
    }

def reference(A_x, A_wqkv, A_wo, B_x, B_w_gate, B_w_up, B_w_down):
    def _A_ref(x, wqkv, wo):
        B, S, D = x.shape
        H = 32; Dh = D // H
        qkv = (lambda x, *d: x.transpose(*d))((x @ wqkv).reshape(B, S, 3, H, Dh), 2, 0, 3, 1, 4)
        q, k, v = qkv[0], qkv[1], qkv[2]
        scale = Dh ** -0.5
        scores = jnp.einsum("bhqd,bhkd->bhqk", q, k) * scale
        p = _softmax(scores, axis=-1)
        o = jnp.einsum("bhqk,bhkd->bhqd", p, v)
        return (lambda x, *d: x.transpose(*d))(o, 0, 2, 1, 3).reshape(B, S, D) @ wo

    def _B_ref(x, w_gate, w_up, w_down):
        g = _silu(x @ w_gate)
        u = x @ w_up
        return (g * u) @ w_down

    x = A_x
    xn = _layernorm(x, axis=-1)
    return x + _A_ref(xn, A_wqkv, A_wo) + _B_ref(xn, B_w_gate, B_w_up, B_w_down)
```

```python
import functools
import math

import jax
import jax.numpy as jnp
import jax.experimental.pallas as pl
import jax.experimental.pallas.tpu as pltpu

S = 2048
D = 640
H = 32
DH = 20
F = 1536
EPS = 1e-5

TQ = 512
NQ = S // TQ
RC = 512
HPG = 6
NG = 6
VW = 32
FC = 512
QSCALE = (DH ** -0.5) * math.log2(math.e)

_NT = (((1,), (1,)), ((), ()))


def _group_base(g):
    return min(HPG * DH * g, D - 128)


def _kernel(x_ref, wqkv_ref, wo_ref, wg_ref, wu_ref, wd_ref, o_ref,
            xn_scr, k_scr, vt_scr, wk_scr, wqt_scr, wvt_scr, qt_scr,
            s0_scr, s1_scr, m0_scr, m1_scr, ot_scr, h_scr):
    step = pl.program_id(0)

    @pl.when(step == 0)
    def _prepare():
        for g in range(NG):
            b = D + _group_base(g)
            wk_scr[:, 128 * g:128 * (g + 1)] = wqkv_ref[:, b:b + 128]
        wqt_scr[...] = wqkv_ref[:, 0:D].astype(jnp.float32).T.astype(jnp.bfloat16)
        wvt_scr[...] = wqkv_ref[:, 2 * D:3 * D].astype(jnp.float32).T.astype(jnp.bfloat16)

        row = jax.lax.broadcasted_iota(jnp.int32, (VW, RC), 0)

        def chunk(c, carry):
            r0 = pl.multiple_of(c * RC, RC)
            xf = x_ref[pl.ds(r0, RC), :].astype(jnp.float32)
            mu = jnp.mean(xf, axis=-1, keepdims=True)
            xc = xf - mu
            var = jnp.mean(xc * xc, axis=-1, keepdims=True)
            xn = (xc * jax.lax.rsqrt(var + EPS)).astype(jnp.bfloat16)
            xn_scr[pl.ds(r0, RC), :] = xn
            kc = jnp.dot(xn, wk_scr[...], preferred_element_type=jnp.float32)
            for g in range(NG):
                k_scr[g, pl.ds(r0, RC), :] = kc[:, 128 * g:128 * (g + 1)].astype(jnp.bfloat16)
            vt = jax.lax.dot_general(wvt_scr[...], xn, _NT,
                                     preferred_element_type=jnp.float32)
            for h in range(H):
                w0 = (DH * h) // 16 * 16
                off = DH * h - w0
                win = vt[w0:w0 + VW, :]
                keep = jnp.logical_and(row >= off, row < off + DH)
                vt_scr[h, :, pl.ds(r0, RC)] = jnp.where(keep, win, 1.0).astype(jnp.bfloat16)
            return carry

        jax.lax.fori_loop(0, S // RC, chunk, 0)

    q0 = pl.multiple_of(step * TQ, TQ)
    xn_blk = xn_scr[pl.ds(q0, TQ), :]
    qt_scr[...] = jax.lax.dot_general(
        wqt_scr[...], xn_blk, _NT, preferred_element_type=jnp.float32) * QSCALE

    row128 = jax.lax.broadcasted_iota(jnp.int32, (128, TQ), 0)
    row32 = jax.lax.broadcasted_iota(jnp.int32, (VW, TQ), 0)

    def scores(h, s_scr, m_scr):
        g = h // HPG
        base = jnp.minimum(HPG * DH * g, D - 128)
        off = DH * h - base
        base = pl.multiple_of(base, 8)
        keep = jnp.logical_and(row128 >= off, row128 < off + DH)
        qm = jnp.where(keep, qt_scr[pl.ds(base, 128), :], 0.0).astype(jnp.bfloat16)
        st = jnp.dot(k_scr[g], qm, preferred_element_type=jnp.float32)
        s_scr[...] = st
        m_scr[...] = jnp.max(st, axis=0, keepdims=True)

    def values(h, s_scr, m_scr):
        p = jnp.exp2(s_scr[...] - m_scr[...]).astype(jnp.bfloat16)
        ow = jnp.dot(vt_scr[h], p, preferred_element_type=jnp.float32)
        w0 = (DH * h) // 16 * 16
        off = DH * h - w0
        w0 = pl.multiple_of(w0, 16)
        denom = jnp.where(off == 12, ow[0:1, :], ow[VW - 1:VW, :])
        on = ow / denom
        keep = jnp.logical_and(row32 >= off, row32 < off + DH)
        pltpu.store(ot_scr.at[pl.ds(w0, VW), :], on, mask=keep)

    scores(0, s0_scr, m0_scr)

    def pair(j, carry):
        h = 2 * j
        scores(h + 1, s1_scr, m1_scr)
        values(h, s0_scr, m0_scr)
        scores(h + 2, s0_scr, m0_scr)
        values(h + 1, s1_scr, m1_scr)
        return carry

    jax.lax.fori_loop(0, H // 2 - 1, pair, 0)
    scores(H - 1, s1_scr, m1_scr)
    values(H - 2, s0_scr, m0_scr)
    values(H - 1, s1_scr, m1_scr)

    for c in range(F // FC):
        gt = jnp.dot(xn_blk, wg_ref[:, FC * c:FC * (c + 1)], preferred_element_type=jnp.float32)
        up = jnp.dot(xn_blk, wu_ref[:, FC * c:FC * (c + 1)], preferred_element_type=jnp.float32)
        h_scr[:, FC * c:FC * (c + 1)] = (gt * jax.nn.sigmoid(gt) * up).astype(jnp.bfloat16)

    o = ot_scr[...].T.astype(jnp.bfloat16)
    attn = jnp.dot(o, wo_ref[...], preferred_element_type=jnp.float32)
    ffn = jnp.dot(h_scr[...], wd_ref[...], preferred_element_type=jnp.float32)
    res = x_ref[pl.ds(q0, TQ), :].astype(jnp.float32)
    o_ref[...] = (res + attn + ffn).astype(o_ref.dtype)


@jax.jit
def pallas_parallel_sum__softmax_full_mha__swiglu_ffn__prompt_kernel(
    A_x: jax.Array,
    A_wqkv: jax.Array,
    A_wo: jax.Array,
    B_x: jax.Array,
    B_w_gate: jax.Array,
    B_w_up: jax.Array,
    B_w_down: jax.Array,
):
    del B_x
    x = A_x.reshape(S, D)
    full = lambda shape: pl.BlockSpec(shape, lambda i: (0,) * len(shape))
    bf16, f32 = jnp.bfloat16, jnp.float32
    out = pl.pallas_call(
        _kernel,
        grid=(NQ,),
        in_specs=[
            full((S, D)), full((D, 3 * D)), full((D, D)),
            full((D, F)), full((D, F)), full((F, D)),
        ],
        out_specs=pl.BlockSpec((TQ, D), lambda i: (i, 0)),
        out_shape=jax.ShapeDtypeStruct((S, D), A_x.dtype),
        scratch_shapes=[
            pltpu.VMEM((S, D), bf16),
            pltpu.VMEM((NG, S, 128), bf16),
            pltpu.VMEM((H, VW, S), bf16),
            pltpu.VMEM((D, NG * 128), bf16),
            pltpu.VMEM((D, D), bf16),
            pltpu.VMEM((D, D), bf16),
            pltpu.VMEM((D, TQ), f32),
            pltpu.VMEM((S, TQ), f32),
            pltpu.VMEM((S, TQ), f32),
            pltpu.VMEM((1, TQ), f32),
            pltpu.VMEM((1, TQ), f32),
            pltpu.VMEM((D, TQ), f32),
            pltpu.VMEM((TQ, F), bf16),
        ],
        compiler_params=pltpu.CompilerParams(
            dimension_semantics=("arbitrary",),
            vmem_limit_bytes=100 * 1024 * 1024,
        ),
    )(x, A_wqkv, A_wo, B_w_gate, B_w_up, B_w_down)
    return out.reshape(A_x.shape)
```

```python
import math

import jax
import jax.numpy as jnp
import jax.experimental.pallas as pl
import jax.experimental.pallas.tpu as pltpu

S = 2048
D = 640
H = 32
DH = 20
F = 1536
EPS = 1e-5

TQ = 512
NQB = S // TQ
NT = TQ // 128
KC = 128
NCH = S // KC
RC = 512
LNB = 32
RB = TQ
OR = 128
HPG = 6
NG = 6
VW = 24
NV = 320
NMX = S - NV
NFULL = NMX // KC
EXTRA = NMX - NFULL * KC
X0 = 3
XS = 3
FILL_FROM = 2
FSLOT = 4
DG = 2
FR = S // (H // 2)
FP = 256
QSCALE = (DH ** -0.5) * math.log2(math.e)
L_MIN = 2.0 ** -60
A_MAX = 2.0 ** 120

KB0 = (0, NV)
QC0 = (2 * NV, 2 * NV + S // 16)
SINK = 2 * NV + S // 8
VPU_ROWS = SINK + 8

_NT = (((1,), (1,)), ((), ()))


def _group_base(g):
    return min(HPG * DH * g, D - 128)


def _rev16(v):
    n = v.shape[0] // 16
    return jnp.concatenate([v[16 * i:16 * (i + 1)] for i in reversed(range(n))], axis=0)


def _fold_max(v):
    r = v[0:8]
    for i in range(1, v.shape[0] // 8):
        r = jnp.maximum(r, v[8 * i:8 * (i + 1)])
    return r


def _kernel(x_hbm, wqkv_hbm, wo_hbm, wg_hbm, wu_hbm, wd_hbm, o_hbm,
            x_ref, wqkv_ref, wo_ref, wg_ref, wu_ref, wd_ref, o_ref, in_sem, out_sem,
            xn_scr, k_scr, vt_scr, wk_scr, wqvt_scr, qt_scr, ot_scr, ob_scr, y_scr, h_scr,
            wgp_scr, wup_scr, wdp_scr, kf_scr, vpu, pv0_scr, pv1_scr, kc_scr, vc_scr,
            amax_scr, dmin_scr, s_scr, z_scr):
    f32, bf16, u32 = jnp.float32, jnp.bfloat16, jnp.uint32
    z_scr[0] = 0
    z_scr[1] = 0

    nxc = S // RC

    def x_copy(c):
        return pltpu.make_async_copy(x_hbm.at[pl.ds(RC * c, RC), :],
                                     x_ref.at[pl.ds(RC * c, RC), :], in_sem.at[c])

    def w_copy(part):
        cols = pl.ds(D * part, D)
        return pltpu.make_async_copy(wqkv_hbm.at[:, cols], wqkv_ref.at[:, cols],
                                     in_sem.at[nxc + part])

    late = [
        pltpu.make_async_copy(wg_hbm, wg_ref, in_sem.at[nxc + 3]),
        pltpu.make_async_copy(wu_hbm, wu_ref, in_sem.at[nxc + 4]),
        pltpu.make_async_copy(wd_hbm, wd_ref, in_sem.at[nxc + 5]),
        pltpu.make_async_copy(wo_hbm, wo_ref, in_sem.at[nxc + 6]),
    ]

    x_copy(0).start()
    w_copy(1).start()
    for c in (3, 1, 2):
        x_copy(c).start()
    w_copy(0).start()
    w_copy(2).start()
    for cp in late:
        cp.start()

    amax_scr[...] = jnp.zeros_like(amax_scr)
    dmin_scr[...] = jnp.ones_like(dmin_scr)

    ln_mask = jax.lax.broadcasted_iota(jnp.int32, (LNB, 1), 0) >= z_scr[1]

    def layernorm(r0, r1, paced=True):
        link = None
        step = LNB if paced else r1 - r0
        for b0 in range(r0, r1, step):
            xf = x_ref[b0:b0 + step, :].astype(f32)
            mu = jnp.mean(xf, axis=-1, keepdims=True)
            if link is not None:
                mu = jnp.where(ln_mask, mu, link)
            xc = xf - mu
            var = jnp.mean(xc * xc, axis=-1, keepdims=True)
            link = jax.lax.rsqrt(var + EPS)
            xn_scr[b0:b0 + step, :] = (xc * link).astype(bf16)

    def store_k(g, r0, tile):
        n = tile.shape[0]
        tile = jnp.concatenate(
            [_rev16(tile[KC * i:KC * (i + 1)]) for i in range(n // KC)], axis=0)
        k_scr[g, r0 // 2:(r0 + n) // 2, :] = pltpu.bitcast(tile.astype(bf16), u32)

    def kproj(c, groups=tuple(range(NG))):
        rows = slice(RC * c, RC * (c + 1))
        kc = jnp.dot(xn_scr[rows, :], wk_scr[:, 128 * groups[0]:128 * (groups[-1] + 1)],
                     preferred_element_type=f32)
        for n, g in enumerate(groups):
            store_k(g, RC * c, kc[:, 128 * n:128 * (n + 1)])
        if c == nxc - 1:
            for h in range(H):
                g = h // HPG
                off = DH * h - _group_base(g)
                tile = kc[RC - NV:, 128 * g:128 * (g + 1)]
                kf_scr[h] = tile if off == 0 else pltpu.roll(tile, 128 - off, 1)

    half = RC // 2
    x_copy(0).wait()
    layernorm(0, half, False)
    w_copy(1).wait()
    wal = jnp.concatenate([wqkv_ref[:, D:D + 128], wqkv_ref[:, 2 * D - 128:2 * D]], axis=1)
    for r0 in (0, half):
        ka = jnp.dot(xn_scr[r0:r0 + half, :], wal, preferred_element_type=f32)
        store_k(0, r0, ka[:, 0:128])
        store_k(NG - 1, r0, ka[:, 128:256])
        if r0 == 0:
            layernorm(half, RC, False)
    for g in range(NG):
        b = D + _group_base(g)
        wk_scr[:, 128 * g:128 * (g + 1)] = wqkv_ref[:, b:b + 128]
    x_copy(3).wait()
    kproj(0, tuple(range(1, NG - 1)))
    layernorm(3 * RC, 4 * RC)
    x_copy(1).wait()
    x_copy(2).wait()
    kproj(3)
    layernorm(RC, 2 * RC)
    kproj(1)
    layernorm(2 * RC, 3 * RC)
    w_copy(0).wait()
    w_copy(2).wait()
    wqvt_scr[0:D, :] = wqkv_ref[:, 0:D].astype(f32).T.astype(bf16)
    kproj(2)
    wqvt_scr[D:2 * D, :] = wqkv_ref[:, 2 * D:3 * D].astype(f32).T.astype(bf16)

    rowv = jax.lax.broadcasted_iota(jnp.int32, (VW, RC), 0)

    def chunk(c, carry):
        r0 = pl.multiple_of(c * RC, RC)
        xn = xn_scr[pl.ds(r0, RC), :]
        qt = jax.lax.dot_general(wqvt_scr[0:D, :], xn, _NT, preferred_element_type=f32) * QSCALE
        for lt in range(RC // 128):
            qt_scr[c * (RC // 128) + lt] = qt[:, 128 * lt:128 * (lt + 1)]
        vt = jax.lax.dot_general(wqvt_scr[D:2 * D, :], xn, _NT, preferred_element_type=f32)
        pad = jnp.zeros((32 - VW, RC), f32)
        for h in range(H):
            w0 = DH * h // 8 * 8
            off = DH * h - w0
            keep = jnp.logical_and(rowv >= off, rowv < off + DH)
            win = jnp.concatenate([jnp.where(keep, vt[w0:w0 + VW, :], 1.0), pad], axis=0)
            vt_scr[h, :, pl.ds(r0, RC)] = pltpu.bitcast(win.astype(bf16), u32)
        return carry

    jax.lax.fori_loop(0, nxc - 2, chunk, 0)
    for cp in late:
        cp.wait()
    chunk(nxc - 2, 0)

    row128 = jax.lax.broadcasted_iota(jnp.int32, (128, TQ), 0)
    units = [(r0, lt) for r0 in range(0, NV // 8, 2) for lt in range(NT)]
    pvs = (pv0_scr, pv1_scr)

    def put_result(item, zw, sink):
        slot, row, val = item
        pvs[slot][pl.ds(zw + row, 8), :] = val
        vpu[0, pl.ds(sink, 8), :] = val

    def masked_q(h, qb):
        g = h // HPG
        base = jnp.minimum(HPG * DH * g, D - 128)
        off = DH * h - base
        base = pl.multiple_of(base, 8)
        keep = jnp.logical_and(row128 >= off, row128 < off + DH)
        qwin = jnp.concatenate(
            [qt_scr[NT * qb + i, pl.ds(base, 128), :] for i in range(NT)], axis=1)
        return jnp.where(keep, qwin, 0.0).astype(bf16)

    def store_head(h, qb, acc):
        ot_scr[qb, pl.ds(pl.multiple_of(VW * h, 8), VW), :] = acc

    def copy_k(g):
        n0 = KC * (X0 - 1) // 2
        kc_scr[0:n0, :] = k_scr[g, 0:n0, :]
        if EXTRA:
            e0 = (KC * (NFULL + 1) - EXTRA) // 2
            kc_scr[n0:n0 + EXTRA // 2, :] = k_scr[g, e0:e0 + EXTRA // 2, :]
        n1 = KC * NFULL // 2 - n0
        kc_scr[n0 + EXTRA // 2:n0 + EXTRA // 2 + n1, :] = k_scr[g, n0:n0 + n1, :]

    def q_rows(h):
        w0 = DH * h // 8 * 8
        return [pl.multiple_of(w0 + 8 * n, 8) for n in range(VW // 8)]

    def fill_q(starts, odd, i, ds=range(DH)):
        for d in ds:
            r = 4 * odd + d
            rows = qt_scr[i, pl.ds(starts[r // 8], 8), :]
            q0 = QC0[odd] + 8 * i
            vpu[d, q0:q0 + 8, :] = jnp.broadcast_to(rows[r % 8:r % 8 + 1], (8, 128))

    def fill_group(h, odd, r, ds=range(DH)):
        kblk = kf_scr[h, 8 * r:8 * (r + 1), :]
        for d in ds:
            k0 = KB0[odd] + 8 * r
            vpu[d, k0:k0 + 8, :] = jnp.broadcast_to(kblk[:, d:d + 1], (8, 128))

    def vpu_block(odd, qb, slot, unit, prev, mask):
        r0, lt = unit
        k0 = KB0[odd] + 8 * r0
        q0 = QC0[odd] + 8 * (NT * qb + lt)
        sv = None
        for d0 in range(0, DH, DG):
            qv = vpu[d0:d0 + DG, q0:q0 + 8, :]
            prod = vpu[d0:d0 + DG, k0:k0 + 16, :] * jnp.concatenate([qv, qv], axis=1)
            if sv is None:
                sv = prod[0] + prod[1]
                if prev is not None:
                    sv = jnp.where(mask, sv, prev)
            else:
                sv = jnp.sum(jnp.concatenate([sv[None], prod], axis=0), axis=0)
        pe = jnp.exp2(sv).astype(bf16)
        return sv, (slot, lt * (NV // 2) + 4 * r0, pltpu.bitcast(pe, f32))

    def load_p32(slot, r0, rows):
        tiles = []
        for i in range(NT):
            b = i * (NV // 2)
            tiles.append(pvs[slot][b + r0 // 2:b + (r0 + rows) // 2, :])
        return jnp.concatenate(tiles, axis=1)

    zw0 = pl.multiple_of(z_scr[0], 8)
    sink0 = pl.multiple_of(zw0 + SINK, 8)
    mask16 = jax.lax.broadcasted_iota(jnp.int32, (16, 128), 0) >= z_scr[1]
    for i in range(NT):
        fill_q(q_rows(0), 0, i)
    prev0, item0 = None, None
    for n, unit in enumerate(units):
        if n % NT == 0:
            for r in ((0, 1, 2, 3) if n == 0 else (unit[0] + 2, unit[0] + 3)):
                if r < NV // 8:
                    fill_group(0, 0, r)
        prev0, item = vpu_block(0, 0, 0, unit, prev0, mask16)
        if item0 is not None:
            put_result(item0, zw0, sink0)
        item0 = item
    put_result(item0, zw0, sink0)

    mask0 = jax.lax.broadcasted_iota(jnp.int32, (8, 128), 0) >= z_scr[1]
    one = jnp.where(mask0, 1.0, 0.0)
    pace = jnp.where(mask0, one, prev0[0:8])
    for w_src, w_dst in ((wg_ref, wgp_scr), (wu_ref, wup_scr), (wd_ref, wdp_scr)):
        rows, cols = w_src.shape
        for r in range(rows // 16):
            for cc in range(cols // 128):
                tile = pltpu.bitcast(w_src[16 * r:16 * (r + 1), 128 * cc:128 * (cc + 1)], u32)
                pace = pace * one * one * one
                tile = jnp.where(mask0, tile, pltpu.bitcast(pace, u32))
                w_dst[8 * r:8 * (r + 1), 128 * cc:128 * (cc + 1)] = tile

    chunk(nxc - 1, 0)
    for i in range(NT, S // 128):
        fill_q(q_rows(0), 0, i)

    def heads(j, carry):
        @pl.when(j % (HPG // 2) == 0)
        def _():
            copy_k(j // (HPG // 2))

        zw = pl.multiple_of(z_scr[0], 8)
        sink = pl.multiple_of(zw + SINK, 8)
        vc_scr[pl.ds(zw, 16), :] = vt_scr[2 * j]
        vc_scr[pl.ds(zw + 16, 16), :] = vt_scr[2 * j + 1]
        mask = jax.lax.broadcasted_iota(jnp.int32, (16, 128), 0) >= z_scr[1]
        hs = [2 * j, 2 * j + 1, jnp.bitwise_and(2 * j + 2, H - 1)]
        qstarts = (q_rows(hs[2]), q_rows(hs[1]))
        nst = 2 * NQB
        pend, accs, left = {}, {}, {}
        delayed = []
        ngrp = NV // 8

        def pv_step(t, c, p):
            odd = t // NQB
            lhs = pltpu.bitcast(vc_scr[16 * odd:16 * (odd + 1), KC * c:KC * (c + 1)], bf16)
            pv = jnp.dot(lhs, p, preferred_element_type=f32)[0:VW]
            accs[t] = pv if t not in accs else accs[t] + pv

        def flush(n):
            while len(delayed) > n:
                put_result(delayed.pop(0), zw, sink)

        def finish(t):
            odd, qb = t // NQB, t % NQB
            acc = accs.pop(t)
            den8 = acc[0:8] if odd else acc[VW - 8:VW]
            store_head(hs[odd], qb, acc)
            amax_scr[...] = jnp.maximum(amax_scr[...], _fold_max(jnp.abs(acc)))
            dmin_scr[odd] = jnp.minimum(dmin_scr[odd], den8)

        fr0 = pl.multiple_of(j * FR, FR)
        xr = xn_scr[pl.ds(fr0, FR), :]
        down_cols = ((0, 256), (256, 512), (512, D))

        def ffn_piece(p):
            if p < F // FP:
                cols = slice(FP * p, FP * (p + 1))
                gt = jnp.dot(xr, pltpu.bitcast(wgp_scr[:, cols], bf16), preferred_element_type=f32)
                up = jnp.dot(xr, pltpu.bitcast(wup_scr[:, cols], bf16), preferred_element_type=f32)
                hg = 0.5 * gt
                hv = pltpu.bitcast((hg * (1.0 + jnp.tanh(hg)) * up).astype(bf16), u32)
                h_scr[pl.ds(zw, FR // 2), cols] = hv
            else:
                lo, hi = down_cols[p - F // FP]
                ffn = jnp.dot(pltpu.bitcast(h_scr[...], bf16),
                              pltpu.bitcast(wdp_scr[:, lo:hi], bf16),
                              preferred_element_type=f32)
                y_scr[pl.ds(fr0, FR), lo:hi] = x_ref[pl.ds(fr0, FR), lo:hi].astype(f32) + ffn

        state = dict(prev=None, blk=0, fill=0)

        def vpu_work(t, want):
            tn = t + 1
            odd_n, qb_n = (tn // NQB) % 2, tn % NQB
            while state["blk"] < want:
                state["prev"], item = vpu_block(
                    odd_n, qb_n, tn % 2, units[state["blk"]], state["prev"], mask)
                delayed.append(item)
                flush(1)
                state["blk"] += 1
                if t < NQB - 1:
                    span, pos, hf, of = (NQB - 1), t, hs[1], 1
                elif t < nst - 1:
                    span, pos, hf, of = NQB, t - (NQB - 1), hs[2], 0
                else:
                    continue
                nitem = (ngrp + S // 128) * DH
                tot = span * len(units) - FILL_FROM - 4
                cur = pos * len(units) + state["blk"] - FILL_FROM
                wantf = min(nitem, max(0, cur) * nitem // tot)
                while state["fill"] < wantf:
                    n, d = divmod(state["fill"], DH)
                    if n < S // 128:
                        fill_q(qstarts[of], of, n, (d,))
                    else:
                        fill_group(hf, of, n - S // 128, (d,))
                    state["fill"] += 1

        ffn_piece(0)
        nslot = NFULL + FSLOT
        for t in range(nst):
            odd, qb = t // NQB, t % NQB
            qm = masked_q(hs[odd], qb)
            state["blk"] = 0
            if t in (0, NQB - 1):
                state["fill"] = 0
            for c in range(NFULL + 1):
                if c < NFULL:
                    xrw = EXTRA if c == X0 - 2 else 0
                    r0 = KC * c + (EXTRA if c > X0 - 2 else 0)
                    kk = pltpu.bitcast(kc_scr[r0 // 2:(r0 + KC + xrw) // 2, :], bf16)
                    st = jnp.dot(kk, qm, preferred_element_type=f32)
                    pend[c] = jnp.exp2(_rev16(st[0:KC])).astype(bf16)
                    if xrw:
                        left[t] = pltpu.bitcast(jnp.exp2(_rev16(st[KC:])).astype(bf16), f32)
                else:
                    ffn_piece(t + 1)
                    vpu_work(t, len(units))
                if c >= 1:
                    cb = c - 1
                    pv_step(t, cb, pend.pop(cb))
                    for n, c2 in enumerate(range(NFULL, NCH)):
                        if cb == X0 - 1 + XS * n:
                            if n == 0 and EXTRA:
                                p32 = jnp.concatenate(
                                    [left.pop(t), load_p32(t % 2, 0, KC - EXTRA)], axis=0)
                            else:
                                p32 = load_p32(t % 2, KC * n - EXTRA, KC)
                            pv_step(t, c2, pltpu.bitcast(p32, bf16))
                if c < NFULL:
                    vpu_work(t, (c + 1) * len(units) // nslot)
            finish(t)
        flush(0)
        return carry

    jax.lax.fori_loop(0, H // 2, heads, 0)

    dmin = jnp.minimum(dmin_scr[0, 7:8, :], dmin_scr[1, 0:1, :])
    ok = jnp.logical_and(amax_scr[...] <= A_MAX, dmin >= L_MIN)
    unsafe = jnp.max(jnp.where(ok, 0.0, 1.0)) > 0.0

    @pl.when(unsafe)
    def _exact():
        def one_stage(i, carry):
            h = i // NQB
            qb = i % NQB
            g = h // HPG
            qm = masked_q(h, qb)

            def score(c, mx):
                k0 = pl.multiple_of(c * (KC // 2), 8)
                kk = pltpu.bitcast(k_scr[g, pl.ds(k0, KC // 2), :], bf16)
                st = _rev16(jnp.dot(kk, qm, preferred_element_type=f32))
                s_scr[c] = st
                return jnp.maximum(mx, _fold_max(st))

            mx = jax.lax.fori_loop(0, NCH, score, jnp.full((8, TQ), -jnp.inf, f32))
            m = jnp.max(mx, axis=0, keepdims=True)

            def weigh(c, acc):
                p = jnp.exp2(s_scr[c] - m).astype(bf16)
                lhs = pltpu.bitcast(vt_scr[h, :, pl.ds(pl.multiple_of(c * KC, KC), KC)], bf16)
                return acc + jnp.dot(lhs, p, preferred_element_type=f32)[0:VW]

            acc = jax.lax.fori_loop(0, NCH, weigh, jnp.zeros((VW, TQ), f32))
            store_head(h, qb, acc)
            return carry

        jax.lax.fori_loop(0, H * NQB, one_stage, 0)

    def out_copy(i):
        r0 = pl.multiple_of(i * OR, OR)
        return pltpu.make_async_copy(o_ref.at[pl.ds(r0, OR), :], o_hbm.at[pl.ds(r0, OR), :],
                                     out_sem.at[i])

    row8 = jax.lax.broadcasted_iota(jnp.int32, (8, RB), 0)

    def block(i, carry):
        parts = []
        for hp in range(H // 2):
            wins = []
            for h, r in ((2 * hp, VW - 1), (2 * hp + 1, 0)):
                win = ot_scr[i, VW * h:VW * (h + 1), :]
                den = jnp.broadcast_to(win[r:r + 1], (8, RB))
                r0 = pl.reciprocal(den, approx=True)
                rcp = r0 * (2.0 - den * r0)
                wins.append([win[8 * n:8 * (n + 1)] * rcp for n in range(VW // 8)])
            ev, od = wins
            parts += [ev[0], ev[1], jnp.where(row8 < 4, ev[2], od[0]), od[1], od[2]]
        ot = jnp.concatenate(parts, axis=0)
        ob_scr[...] = pltpu.bitcast(ot.T.astype(bf16), u32)
        for s in range(RB // OR):
            r0 = pl.multiple_of(i * RB + s * OR, OR)
            lhs = pltpu.bitcast(ob_scr[s * OR // 2:(s + 1) * OR // 2, :], bf16)
            attn = jnp.dot(lhs, wo_ref[...], preferred_element_type=f32)
            o_ref[pl.ds(r0, OR), :] = (y_scr[pl.ds(r0, OR), :] + attn).astype(o_ref.dtype)
            out_copy(i * (RB // OR) + s).start()
        return carry

    jax.lax.fori_loop(0, S // RB, block, 0)
    for i in range(S // OR):
        out_copy(i).wait()


@jax.jit
def pallas_parallel_sum__softmax_full_mha__swiglu_ffn__prompt_kernel(
    A_x: jax.Array,
    A_wqkv: jax.Array,
    A_wo: jax.Array,
    B_x: jax.Array,
    B_w_gate: jax.Array,
    B_w_up: jax.Array,
    B_w_down: jax.Array,
):
    del B_x
    x = A_x.reshape(S, D)
    bf16, f32, u32 = jnp.bfloat16, jnp.float32, jnp.uint32
    out = pl.pallas_call(
        _kernel,
        out_shape=jax.ShapeDtypeStruct((S, D), A_x.dtype),
        in_specs=[pl.BlockSpec(memory_space=pl.ANY)] * 6,
        out_specs=pl.BlockSpec(memory_space=pl.ANY),
        scratch_shapes=[
            pltpu.VMEM((S, D), bf16),
            pltpu.VMEM((D, 3 * D), bf16),
            pltpu.VMEM((D, D), bf16),
            pltpu.VMEM((D, F), bf16),
            pltpu.VMEM((D, F), bf16),
            pltpu.VMEM((F, D), bf16),
            pltpu.VMEM((S, D), bf16),
            pltpu.SemaphoreType.DMA((S // RC + 7,)),
            pltpu.SemaphoreType.DMA((S // OR,)),
            pltpu.VMEM((S, D), bf16),
            pltpu.VMEM((NG, S // 2, 128), u32),
            pltpu.VMEM((H, 16, S), u32),
            pltpu.VMEM((D, NG * 128), bf16),
            pltpu.VMEM((2 * D, D), bf16),
            pltpu.VMEM((S // 128, D, 128), f32),
            pltpu.VMEM((NQB, H * VW, TQ), f32),
            pltpu.VMEM((RB // 2, D), u32),
            pltpu.VMEM((S, D), f32),
            pltpu.VMEM((FR // 2, F), u32),
            pltpu.VMEM((D // 2, F), u32),
            pltpu.VMEM((D // 2, F), u32),
            pltpu.VMEM((F // 2, D), u32),
            pltpu.VMEM((H, NV, 128), f32),
            pltpu.VMEM((DH, VPU_ROWS, 128), f32),
            pltpu.VMEM((NT * NV // 2, 128), f32),
            pltpu.VMEM((NT * NV // 2, 128), f32),
            pltpu.VMEM((NMX // 2, 128), u32),
            pltpu.VMEM((32, S), u32),
            pltpu.VMEM((8, TQ), f32),
            pltpu.VMEM((2, 8, TQ), f32),
            pltpu.VMEM((NCH, KC, TQ), f32),
            pltpu.SMEM((2,), jnp.int32),
        ],
        compiler_params=pltpu.CompilerParams(
            vmem_limit_bytes=110 * 1024 * 1024,
        ),
    )(x, A_wqkv, A_wo, B_w_gate, B_w_up, B_w_down)
    return out.reshape(A_x.shape)
```
